```python
import jax
import jax.numpy as jnp

def _softmax(x, axis=-1):
    return jax.nn.softmax(x, axis=axis)

def _gelu(x):
    return jax.nn.gelu(x, approximate=True)

def _silu(x):
    return jax.nn.silu(x)

def _sigmoid(x):
    return jax.nn.sigmoid(x)

def _layernorm(x, axis=-1, eps=1e-05):
    m = jnp.mean(x, axis=axis, keepdims=True)
    v = jnp.var(x, axis=axis, keepdims=True)
    return (x - m) / jnp.sqrt(v + eps)

def _scatter_add(tgt, idx, src, axis=0):
    return tgt.at[idx].add(src)

def _segment_sum(src, seg, n):
    return jax.ops.segment_sum(src, seg, n)

class _Rng:

    def __init__(self, key):
        self._k = key

    def _next(self):
        self._k, sub = jax.random.split(self._k)
        return sub

    def normal(self, shape):
        return jax.random.normal(self._next(), shape, dtype=jnp.bfloat16)

    def randint(self, lo, hi, shape):
        return jax.random.randint(self._next(), shape, lo, hi, dtype=jnp.int32)

    def uniform(self, shape, lo=0.0, hi=1.0):
        return jax.random.uniform(self._next(), shape, jnp.bfloat16, lo, hi)

    def permutation(self, n):
        return jax.random.permutation(self._next(), n)
kernel_name = 'adaLN_cond__gqa_block_cached__moe_arch_mod__prompt'

def setup_inputs():
    _rng = _Rng(jax.random.key(int.from_bytes(__import__("os").urandom(4), "little")))
    _w = lambda a: (lambda t: t.astype(jnp.bfloat16) if jnp.issubdtype(t.dtype, jnp.floating) else t)(jnp.asarray(a))

    def _A_setup():
        B, Sq, D = (1, 2048, 576)
        Hq, Hkv, Sk, Dh = (32, 16, 2048, 128)
        assert Hq % Hkv == 0, (Hq, Hkv)
        return {'x': _w((lambda *s: _rng.normal(s) * 0.05)(B, Sq, D)), 'k_cache': _w((lambda *s: _rng.normal(s) * 0.05)(B, Hkv, Sk, Dh)), 'v_cache': _w((lambda *s: _rng.normal(s) * 0.05)(B, Hkv, Sk, Dh)), 'wq': _w((lambda *s: _rng.normal(s) * 0.05)(D, Hq * Dh) * D ** (-0.5)), 'wo': _w((lambda *s: _rng.normal(s) * 0.05)(Hq * Dh, D) * (Hq * Dh) ** (-0.5))}
    _A_in = _A_setup()

    def _B_setup():
        B, S, D, F, C = (1, 2048, 576, 4608, 8)
        return {'x': _w((lambda *s: _rng.normal(s) * 0.05)(B, S, D)), 'w_r': _w((lambda *s: _rng.normal(s) * 0.05)(D)), 'w_gate': _w((lambda *s: _rng.normal(s) * 0.05)(D, F)), 'w_up': _w((lambda *s: _rng.normal(s) * 0.05)(D, F)), 'w_down': _w((lambda *s: _rng.normal(s) * 0.05)(F, D))}
    _B_in = _B_setup()
    return {'A_x': _A_in['x'], 'A_k_cache': _A_in['k_cache'], 'A_v_cache': _A_in['v_cache'], 'A_wq': _A_in['wq'], 'A_wo': _A_in['wo'], 'B_x': _B_in['x'], 'B_w_r': _B_in['w_r'], 'B_w_gate': _B_in['w_gate'], 'B_w_up': _B_in['w_up'], 'B_w_down': _B_in['w_down'], 'c': _w((lambda *s: _rng.normal(s) * 0.05)(1, 576)), 'w_mod': _w((lambda *s: _rng.normal(s) * 0.05)(576, 6 * 576) * 576 ** (-0.5))}

def reference(A_x, A_k_cache, A_v_cache, A_wq, A_wo, B_x, B_w_r, B_w_gate, B_w_up, B_w_down, c, w_mod):

    def _A_ref(x, k_cache, v_cache, wq, wo):
        B, Sq, D = x.shape
        Hq, Dh = (32, 128)
        Hkv = k_cache.shape[1]
        rep = Hq // Hkv
        q = (lambda x, *d: x.transpose(*d))((x @ wq).reshape(B, Sq, Hq, Dh), 0, 2, 1, 3)
        k = jnp.repeat(k_cache, rep, axis=1)
        v = jnp.repeat(v_cache, rep, axis=1)
        scores = jnp.einsum('bhqd,bhkd->bhqk', q, k) * Dh ** (-0.5)
        p = _softmax(scores, axis=-1)
        o = jnp.einsum('bhqk,bhkd->bhqd', p, v)
        return (lambda x, *d: x.transpose(*d))(o, 0, 2, 1, 3).reshape(B, Sq, Hq * Dh) @ wo

    def _B_ref(x, w_r, w_gate, w_up, w_down):
        B, S, D = x.shape
        C = 8
        r = x @ w_r
        idx = jnp.argsort(-r, axis=-1)[:, :C]
        idx_e = jnp.repeat(idx.reshape(B, C, 1), D, axis=2)
        x_sel = jnp.take_along_axis(x, idx_e, axis=1)
        g = _silu(x_sel @ w_gate)
        u = x_sel @ w_up
        y = g * u @ w_down
        r_sel = _sigmoid(jnp.take_along_axis(r, idx, axis=1))
        y = y * r_sel.reshape(B, C, 1)
        b_off = (jnp.arange(B) * S).reshape(B, 1)
        flat_idx = (idx + b_off).reshape(B * C)
        zero = (x * 0.0).reshape(B * S, D)
        upd = _scatter_add(zero, flat_idx, y.reshape(B * C, D), axis=0)
        return x + upd.reshape(B, S, D)
    x = A_x
    mod = (_silu(c) @ w_mod).reshape(c.shape[0], 6, 1, -1)
    sa, ca, ga, sb, cb, gb = (mod[:, 0].copy(), mod[:, 1].copy(), mod[:, 2].copy(), mod[:, 3].copy(), mod[:, 4].copy(), mod[:, 5].copy())
    h = _layernorm(x, axis=-1) * (1 + ca) + sa
    x = x + ga * _A_ref(h, A_k_cache, A_v_cache, A_wq, A_wo)
    h = _layernorm(x, axis=-1) * (1 + cb) + sb
    x = x + gb * _B_ref(h, B_w_r, B_w_gate, B_w_up, B_w_down)
    return x
```

```python
import jax
import jax.numpy as jnp
from jax import lax
import jax.experimental.pallas as pl
import jax.experimental.pallas.tpu as pltpu

S = 2048
D = 576
HQ = 32
HKV = 16
DH = 128
F = 4608
C = 8
EPS_BF16 = 1.0013580322265625e-05
QSCALE = DH ** -0.5 * 1.4426950408889634
BF = jnp.bfloat16
F32 = jnp.float32
I32 = jnp.int32

NT = (((1,), (1,)), ((), ()))


def _rnd(x):
    return x.astype(BF).astype(F32)


def _ln_mod_t(x, scale1, shift):
    mean = jnp.sum(x, axis=0, keepdims=True) * (1.0 / D)
    xc = x - mean
    var = jnp.sum(xc * xc, axis=0, keepdims=True) * (1.0 / D)
    den = _rnd(jnp.sqrt(_rnd(_rnd(var) + EPS_BF16)))
    inv = 1.0 / den
    y = _rnd(_rnd(x - _rnd(mean)) * inv)
    y = _rnd(y * scale1)
    return _rnd(y + shift)


def make_kernel(BQ, CK, fuse_special, newton):
    NQB = S // BQ
    U = NQB * HKV
    NL = BQ // 128

    def kernel(xT_hbm, k_hbm, v_hbm, wq_hbm, woT_hbm, wr_hbm, wg_hbm, wu_hbm, wdT_hbm, c_hbm, wm_hbm,
               o_hbm,
               xT_v, k_v, v_v, wq_v, woT_v, wr_v, wg_v, wu_v, wdT_v, c_v, wm_v,
               tab_s, gb_s, h_s, q_s, s_s, acc_s, ls_s, at_s, x1_s, h2_s, out_s, r_s,
               sems, ksem, vsem, qsem, osem):
        cp_c = pltpu.make_async_copy(c_hbm, c_v, sems.at[0])
        cp_wm = pltpu.make_async_copy(wm_hbm, wm_v, sems.at[1])
        cp_x = pltpu.make_async_copy(xT_hbm, xT_v, sems.at[2])
        cp_wr = pltpu.make_async_copy(wr_hbm, wr_v, sems.at[3])
        cp_wg = pltpu.make_async_copy(wg_hbm, wg_v, sems.at[4])
        cp_wu = pltpu.make_async_copy(wu_hbm, wu_v, sems.at[5])
        cp_wd = pltpu.make_async_copy(wdT_hbm, wdT_v, sems.at[6])

        def cp_k(g):
            return pltpu.make_async_copy(k_hbm.at[g], k_v.at[g], ksem.at[g])

        def cp_v(g):
            return pltpu.make_async_copy(v_hbm.at[g], v_v.at[g], vsem.at[g])

        def cp_q(g):
            c0 = pl.multiple_of(g * 256, 256)
            return pltpu.make_async_copy(wq_hbm.at[:, pl.ds(c0, 256)], wq_v.at[:, pl.ds(c0, 256)], qsem.at[g])

        def cp_o(g):
            c0 = pl.multiple_of(g * 256, 256)
            return pltpu.make_async_copy(woT_hbm.at[:, pl.ds(c0, 256)], woT_v.at[:, pl.ds(c0, 256)], osem.at[g])

        cp_c.start()
        cp_wm.start()
        cp_x.start()
        cp_wr.start()
        cp_q(0).start()
        for g in range(HKV):
            cp_k(g).start()
            cp_v(g).start()
            if g + 1 < HKV:
                cp_q(g + 1).start()
            cp_o(g).start()
        cp_wg.start()
        cp_wu.start()
        cp_wd.start()

        cp_c.wait()
        cp_wm.wait()
        cf = c_v[...].astype(F32)
        sc = _rnd(cf * _rnd(jax.nn.sigmoid(cf)))
        sc16 = jnp.broadcast_to(sc, (16, D)).astype(BF)
        mod = _rnd(jnp.dot(sc16, wm_v[...], preferred_element_type=F32)[0:8, :])
        gb_s[...] = mod[:, 5 * D:6 * D]
        modT = jnp.broadcast_to(mod[0:1, :], (128, 6 * D)).T
        tab_s[0 * D:1 * D, :] = modT[0 * D:1 * D]
        tab_s[1 * D:2 * D, :] = _rnd(1.0 + modT[1 * D:2 * D])
        tab_s[2 * D:3 * D, :] = modT[2 * D:3 * D]
        tab_s[3 * D:4 * D, :] = modT[3 * D:4 * D]
        tab_s[4 * D:5 * D, :] = _rnd(1.0 + modT[4 * D:5 * D])
        tab_s[5 * D:6 * D, :] = modT[5 * D:6 * D]
        cp_wr.wait()
        tab_s[6 * D:7 * D, :] = jnp.broadcast_to(wr_v[...].astype(F32), (128, D)).T

        def tab(i):
            t = tab_s[i * D:(i + 1) * D, :]
            return jnp.concatenate([t] * NL, axis=1) if NL > 1 else t

        def ln1(qb):
            c0 = pl.multiple_of(qb * BQ, BQ)
            x = xT_v[:, pl.ds(c0, BQ)].astype(F32)
            hT = _ln_mod_t(x, tab(1), tab(0)).astype(BF)
            h_s[qb % 2] = hT.T

        def qproj(qb, g, slot):
            c0 = pl.multiple_of(g * 256, 256)
            q = jnp.dot(h_s[qb % 2], wq_v[:, pl.ds(c0, 256)], preferred_element_type=F32)
            q_s[slot] = (q * QSCALE).astype(BF)

        def norm(j):
            l = jnp.sum(ls_s[j], axis=-1, keepdims=True)
            if newton:
                r0 = pltpu.reciprocal(l, approx=True)
                r = r0 * (2.0 - l * r0)
            else:
                r = pltpu.reciprocal(l, approx=False)
            return (acc_s[j] * r).astype(BF)

        def oproj(qb, g):
            c0 = pl.multiple_of(g * 256, 256)
            o2 = jnp.concatenate([norm(0), norm(1)], axis=1)
            contrib = lax.dot_general(woT_v[:, pl.ds(c0, 256)], o2, NT, preferred_element_type=F32)
            prev = jnp.where(g == 0, 0.0, at_s[qb % 2])
            at_s[qb % 2] = prev + contrib

        def qk(qh, g, s_ref):
            mx = None
            for c in range(S // CK):
                s = lax.dot_general(qh, k_v[g, pl.ds(c * CK, CK), :], NT, preferred_element_type=F32)
                s_ref[:, pl.ds(c * CK, CK)] = s
                for t in range(CK // 128):
                    st = s[:, t * 128:(t + 1) * 128]
                    mx = st if mx is None else jnp.maximum(mx, st)
            return jnp.max(mx, axis=-1, keepdims=True)

        def pv_raw(g, s_ref, m):
            acc = None
            ls = None
            for c in range(S // CK):
                p = jnp.exp2(s_ref[:, pl.ds(c * CK, CK)] - m)
                tl = [p[:, t * 128:(t + 1) * 128] for t in range(CK // 128)]
                while len(tl) > 1:
                    tl = [tl[i] + tl[i + 1] for i in range(0, len(tl), 2)]
                ls = tl[0] if ls is None else ls + tl[0]
                d = jnp.dot(p.astype(BF), v_v[g, pl.ds(c * CK, CK), :], preferred_element_type=F32)
                acc = d if acc is None else acc + d
            return acc, ls

        def attention(u):
            g = u % HKV
            res = []
            for j in range(2):
                m = qk(q_s[u % 2, :, j * 128:(j + 1) * 128], g, s_s.at[j])
                res.append(pv_raw(g, s_s.at[j], m))
            for j in range(2):
                acc_s[j] = res[j][0]
                ls_s[j] = res[j][1]

        def epilogue(qb):
            c0 = pl.multiple_of(qb * BQ, BQ)
            x = xT_v[:, pl.ds(c0, BQ)].astype(F32)
            x1 = _rnd(x + _rnd(tab(2) * _rnd(at_s[qb % 2])))
            h2 = _ln_mod_t(x1, tab(4), tab(3))
            x1_s[:, pl.ds(c0, BQ)] = x1.astype(BF)
            h2_s[:, pl.ds(c0, BQ)] = h2.astype(BF)
            r = jnp.sum(h2 * tab(6), axis=0, keepdims=True)
            r_s[pl.ds(qb, 1), :] = _rnd(r)
            out_s[:, pl.ds(c0, BQ)] = (x1 + _rnd(tab(5) * h2)).astype(BF)

        cp_x.wait()
        ln1(0)
        cp_q(0).wait()
        qproj(0, 0, 0)
        acc_s[...] = jnp.zeros(acc_s.shape, F32)
        ls_s[...] = jnp.ones(ls_s.shape, F32)
        at_s[...] = jnp.zeros(at_s.shape, F32)

        def unit(u, special):
            qb = u // HKV
            un = jnp.minimum(u + 1, U - 1)
            up = jnp.maximum(u - 1, 0)
            oproj(up // HKV, up % HKV)
            qproj(un // HKV, un % HKV, (u + 1) % 2)
            attention(u)
            if special:
                epilogue(jnp.maximum(qb - 1, 0))
                ln1(jnp.minimum(qb + 1, NQB - 1))

        def body(u, carry):
            g = u % HKV

            @pl.when(u < HKV)
            def _():
                cp_k(g).wait()
                cp_v(g).wait()

                @pl.when(g + 1 < HKV)
                def _():
                    cp_q(g + 1).wait()

                @pl.when(g >= 1)
                def _():
                    cp_o(g - 1).wait()

            @pl.when(u == HKV)
            def _():
                cp_o(HKV - 1).wait()

            if fuse_special:
                @pl.when(g == 1)
                def _():
                    unit(u, True)

                @pl.when(g != 1)
                def _():
                    unit(u, False)
            else:
                unit(u, False)

                @pl.when(g == 1)
                def _():
                    qb = u // HKV
                    epilogue(jnp.maximum(qb - 1, 0))
                    ln1(jnp.minimum(qb + 1, NQB - 1))
            return carry

        lax.fori_loop(0, U, body, 0)
        oproj(NQB - 1, HKV - 1)
        epilogue(NQB - 1)

        r = r_s[...] + 0.0
        pos = lax.broadcasted_iota(I32, (NQB, BQ), 0) * BQ + lax.broadcasted_iota(I32, (NQB, BQ), 1)
        b16 = lax.shift_right_logical(pltpu.bitcast(r, I32), 16)
        o16 = jnp.where(b16 >= 0x8000, 0xFFFF - b16, b16 + 0x8000)
        o16 = jnp.where(r != r, 0, o16)
        key = pltpu.bitcast(0x10000000 | (o16 << 11) | (S - 1 - pos), F32)
        rowc = lax.broadcasted_iota(I32, (16, 1), 0)
        idxcol = jnp.full((16, 1), -1, I32)
        rsel = jnp.zeros((16, 1), F32)
        for i in range(C):
            m = jnp.max(jnp.max(key, axis=1, keepdims=True), axis=0, keepdims=True)
            key = jnp.where(key == m, 0.0, key)
            mb = pltpu.bitcast(m, I32)
            idx = (S - 1) - (mb & (S - 1))
            o = lax.shift_right_logical(mb, 11) & 0xFFFF
            rb = jnp.where(o >= 0x8000, o - 0x8000, 0xFFFF - o)
            rv = pltpu.bitcast(rb << 16, F32)
            idxcol = jnp.where(rowc == i, idx, idxcol)
            rsel = jnp.where(rowc == i, rv, rsel)
        lane = lax.broadcasted_iota(I32, (16, S), 1)
        ohm = lane == idxcol
        oh = jnp.where(ohm, 1.0, 0.0).astype(BF)
        xs = lax.dot_general(oh, h2_s[...], NT, preferred_element_type=F32)
        x1sel = lax.dot_general(oh, x1_s[...], NT, preferred_element_type=F32)
        xsb = xs.astype(BF)
        cp_wg.wait()
        cp_wu.wait()
        cp_wd.wait()
        gt = _rnd(jnp.dot(xsb, wg_v[...], preferred_element_type=F32))
        gg = _rnd(gt * _rnd(jax.nn.sigmoid(gt)))
        uu = _rnd(jnp.dot(xsb, wu_v[...], preferred_element_type=F32))
        a = (gg * uu).astype(BF)
        y = _rnd(lax.dot_general(a, wdT_v[...], NT, preferred_element_type=F32))
        y = _rnd(y * _rnd(jax.nn.sigmoid(rsel)))
        gb_row = jnp.broadcast_to(gb_s[0:1, :], (16, D))
        new = _rnd(x1sel + _rnd(gb_row * _rnd(xs + y)))
        newT = jnp.concatenate([new, jnp.zeros((128 - 16, D), F32)], axis=0).T
        oh128 = jnp.concatenate([oh, jnp.zeros((128 - 16, S), BF)], axis=0)
        patchT = jnp.dot(newT.astype(BF), oh128, preferred_element_type=F32)
        sel = jnp.max(jnp.where(ohm, 1.0, 0.0), axis=0, keepdims=True) > 0.5
        out_s[...] = jnp.where(sel, patchT.astype(BF), out_s[...])
        ocp = pltpu.make_async_copy(out_s, o_hbm, sems.at[0])
        ocp.start()
        ocp.wait()

    return kernel


def run(A_x, A_k_cache, A_v_cache, A_wq, A_wo, B_x, B_w_r, B_w_gate, B_w_up, B_w_down, c, w_mod,
        BQ=256, CK=512, fuse=True, newton=True, flags=None):
    xT = A_x.reshape(S, D).T
    k = A_k_cache.reshape(HKV, S, DH)
    v = A_v_cache.reshape(HKV, S, DH)
    wr = B_w_r.reshape(1, D)
    NQB = S // BQ
    any_spec = pl.BlockSpec(memory_space=pl.ANY)
    outT = pl.pallas_call(
        make_kernel(BQ, CK, fuse, newton),
        in_specs=[any_spec] * 11,
        out_specs=any_spec,
        out_shape=jax.ShapeDtypeStruct((D, S), BF),
        scratch_shapes=[
            pltpu.VMEM((D, S), BF),
            pltpu.VMEM((HKV, S, DH), BF),
            pltpu.VMEM((HKV, S, DH), BF),
            pltpu.VMEM((D, HQ * DH), BF),
            pltpu.VMEM((D, HQ * DH), BF),
            pltpu.VMEM((1, D), BF),
            pltpu.VMEM((D, F), BF),
            pltpu.VMEM((D, F), BF),
            pltpu.VMEM((D, F), BF),
            pltpu.VMEM((1, D), BF),
            pltpu.VMEM((D, 6 * D), BF),
            pltpu.VMEM((7 * D, 128), F32),
            pltpu.VMEM((8, D), F32),
            pltpu.VMEM((2, BQ, D), BF),
            pltpu.VMEM((2, BQ, 256), BF),
            pltpu.VMEM((2, BQ, S), F32),
            pltpu.VMEM((2, BQ, 128), F32),
            pltpu.VMEM((2, BQ, 128), F32),
            pltpu.VMEM((2, D, BQ), F32),
            pltpu.VMEM((D, S), BF),
            pltpu.VMEM((D, S), BF),
            pltpu.VMEM((D, S), BF),
            pltpu.VMEM((NQB, BQ), F32),
            pltpu.SemaphoreType.DMA((7,)),
            pltpu.SemaphoreType.DMA((HKV,)),
            pltpu.SemaphoreType.DMA((HKV,)),
            pltpu.SemaphoreType.DMA((HKV,)),
            pltpu.SemaphoreType.DMA((HKV,)),
        ],
        compiler_params=pltpu.CompilerParams(vmem_limit_bytes=110 * 1024 * 1024, flags=flags),
    )(xT, k, v, A_wq, A_wo.T, wr, B_w_gate, B_w_up, B_w_down.T, c, w_mod)
    return outT.T.reshape(1, S, D)


@jax.jit
def pallas_adaLN_cond__gqa_block_cached__moe_arch_mod__prompt_kernel(
    A_x: jax.Array,
    A_k_cache: jax.Array,
    A_v_cache: jax.Array,
    A_wq: jax.Array,
    A_wo: jax.Array,
    B_x: jax.Array,
    B_w_r: jax.Array,
    B_w_gate: jax.Array,
    B_w_up: jax.Array,
    B_w_down: jax.Array,
    c: jax.Array,
    w_mod: jax.Array,
):
    return run(A_x, A_k_cache, A_v_cache, A_wq, A_wo, B_x, B_w_r, B_w_gate, B_w_up, B_w_down, c, w_mod)
```

```python
import jax
import jax.numpy as jnp
from jax import lax
import jax.experimental.pallas as pl
import jax.experimental.pallas.tpu as pltpu

S = 2048
D = 576
HQ = 32
HKV = 16
DH = 128
F = 4608
C = 8
EPS_BF16 = 1.0013580322265625e-05
QSCALE = DH ** -0.5 * 1.4426950408889634
BF = jnp.bfloat16
F32 = jnp.float32
I32 = jnp.int32

NT = (((1,), (1,)), ((), ()))
DBG = ''
import contextlib
def scope(n):
    return jax.named_scope(n) if 'scope' in DBG else contextlib.nullcontext()


def _rnd(x):
    return x.astype(BF).astype(F32)


def _ln_stats_t(x):
    mean = jnp.sum(x, axis=0, keepdims=True) * (1.0 / D)
    xc = x - mean
    var = jnp.sum(xc * xc, axis=0, keepdims=True) * (1.0 / D)
    return mean, xc, var


def make_kernel(BQ, CK, orders, reps, fuse, gate_j, opaque, pair, split, QCK, mxmode, lsmode, rmxu, NSPL, early, RS, sched):
    NQB = S // BQ
    U = NQB * HKV
    NL = BQ // 128
    WA = 2 * D

    def kernel(xT_hbm, k_hbm, v_hbm, wq_hbm, woT_hbm, wr_hbm, wg_hbm, wu_hbm, wdT_hbm, c_hbm, wm_hbm,
               o_hbm,
               xT_v, k_v, v_v, wq_v, woT_v, wr_v, wg_v, wu_v, wdT_v, c_v, wm_v,
               tab_s, gb_s, wrb_s, h_s, q_s, s_a, s_b, z_s, acc_s, ls_s, at_s, h2_s, out_s, r_s,
               sems, ksem, vsem, qsem, osem, outsem, wsem):
        cp_c = pltpu.make_async_copy(c_hbm, c_v, sems.at[0])
        cp_wma = [pltpu.make_async_copy(wm_hbm.at[pl.ds(i * (D // NSPL), D // NSPL), pl.ds(0, WA)],
                                        wm_v.at[pl.ds(i * (D // NSPL), D // NSPL), pl.ds(0, WA)], wsem.at[i])
                  for i in range(NSPL)]
        cp_wmb = pltpu.make_async_copy(wm_hbm.at[:, pl.ds(WA, 6 * D - WA)], wm_v.at[:, pl.ds(WA, 6 * D - WA)],
                                       sems.at[2])
        cp_x0 = pltpu.make_async_copy(xT_hbm.at[:, pl.ds(0, BQ)], xT_v.at[:, pl.ds(0, BQ)], sems.at[3])
        cp_xr = pltpu.make_async_copy(xT_hbm.at[:, pl.ds(BQ, S - BQ)], xT_v.at[:, pl.ds(BQ, S - BQ)], sems.at[4])
        cp_wr = pltpu.make_async_copy(wr_hbm, wr_v, sems.at[5])
        cp_wg = pltpu.make_async_copy(wg_hbm, wg_v, sems.at[6])
        cp_wu = pltpu.make_async_copy(wu_hbm, wu_v, sems.at[7])
        cp_wd = pltpu.make_async_copy(wdT_hbm, wdT_v, sems.at[8])

        def cp_k(g):
            return pltpu.make_async_copy(k_hbm.at[g], k_v.at[g], ksem.at[g])

        def cp_v(g):
            return pltpu.make_async_copy(v_hbm.at[g], v_v.at[g], vsem.at[g])

        def cp_q(g):
            c0 = pl.multiple_of(g * 256, 256)
            return pltpu.make_async_copy(wq_hbm.at[:, pl.ds(c0, 256)], wq_v.at[:, pl.ds(c0, 256)], qsem.at[g])

        def cp_o(g):
            c0 = pl.multiple_of(g * 256, 256)
            return pltpu.make_async_copy(woT_hbm.at[:, pl.ds(c0, 256)], woT_v.at[:, pl.ds(c0, 256)], osem.at[g])

        def cp_out(qb):
            c0 = pl.multiple_of(qb * BQ, BQ)
            return pltpu.make_async_copy(out_s.at[:, pl.ds(c0, BQ)], o_hbm.at[:, pl.ds(c0, BQ)], outsem.at[qb])

        def cp_tile(t):
            return pltpu.make_async_copy(out_s.at[:, pl.ds(t * 128, 128)], o_hbm.at[:, pl.ds(t * 128, 128)],
                                         ksem.at[t])

        z_s[0] = 0
        cp_x0.start()
        cp_c.start()
        for cp in cp_wma:
            cp.start()
        if early == 0:
            cp_q(0).start()
            cp_k(0).start()
            cp_v(0).start()

        def col_table(row):
            return jnp.broadcast_to(row, (128, row.shape[1])).T

        _s = scope('pro_mod'); _s.__enter__()

        def tables_b():
            cf = c_v[...].astype(F32)
            sc = _rnd(cf * _rnd(jax.nn.sigmoid(cf)))
            sc16 = jnp.broadcast_to(sc, (16, D)).astype(BF)
            modb = _rnd(jnp.dot(sc16, wm_v[:, WA:6 * D], preferred_element_type=F32)[0:8, :])
            gb_s[...] = modb[:, 3 * D:4 * D]
            tb = col_table(modb[0:1, :])
            tab_s[2 * D:3 * D, :] = tb[0:D]
            tab_s[3 * D:4 * D, :] = tb[D:2 * D]
            tab_s[4 * D:5 * D, :] = _rnd(1.0 + tb[2 * D:3 * D])
            tab_s[5 * D:6 * D, :] = tb[3 * D:4 * D]
            if rmxu:
                wrb_s[...] = jnp.broadcast_to(wr_v[...], (16, D))
            else:
                tab_s[6 * D:7 * D, :] = col_table(wr_v[...].astype(F32))

        def tab(i):
            t = tab_s[i * D:(i + 1) * D, :]
            return jnp.concatenate([t] * NL, axis=1) if NL > 1 else t

        def ln1(qb, mid=None):
            c0 = pl.multiple_of(qb * BQ, BQ)
            x = xT_v[:, pl.ds(c0, BQ)].astype(F32)
            mean, xc, var = _ln_stats_t(x)
            inv = lax.rsqrt(var + 1e-5)
            if mid is not None:
                mid()
            hT = (xc * inv * tab(1) + tab(0)).astype(BF)
            h_s[qb % 2] = hT.T

        def qproj(qb, g, slot):
            c0 = pl.multiple_of(g * 256, 256)
            q = jnp.dot(h_s[qb % 2], wq_v[:, pl.ds(c0, 256)], preferred_element_type=F32)
            q_s[slot] = (q * QSCALE).astype(BF)

        def qproj_half(qb, g, slot, part):
            c0 = pl.multiple_of(g * 256 + part * 128, 128)
            q = jnp.dot(h_s[qb % 2], wq_v[:, pl.ds(c0, 128)], preferred_element_type=F32)
            q_s[slot, :, part * 128:(part + 1) * 128] = (q * QSCALE).astype(BF)

        def qproj_rows(qb, g, slot, part):
            c0 = pl.multiple_of(g * 256, 256)
            rows = slice(part * (BQ // 2), (part + 1) * (BQ // 2))
            q = jnp.dot(h_s[qb % 2, rows], wq_v[:, pl.ds(c0, 256)], preferred_element_type=F32)
            q_s[slot, rows] = (q * QSCALE).astype(BF)

        def oproj_half(qb, g, part):
            c0 = pl.multiple_of(g * 256 + part * 128, 128)
            contrib = lax.dot_general(woT_v[:, pl.ds(c0, 128)], norm(part), NT, preferred_element_type=F32)
            if part == 0:
                prev = jnp.where(g == 0, 0.0, at_s[qb % 2])
            else:
                prev = at_s[qb % 2]
            at_s[qb % 2] = prev + contrib

        def norm(j):
            l = jnp.sum(ls_s[j], axis=-1, keepdims=True)
            r0 = pltpu.reciprocal(l, approx=True)
            r = r0 * (2.0 - l * r0)
            return (acc_s[j] * r).astype(BF)

        def oproj(qb, g):
            c0 = pl.multiple_of(g * 256, 256)
            o2 = jnp.concatenate([norm(0), norm(1)], axis=1)
            contrib = lax.dot_general(woT_v[:, pl.ds(c0, 256)], o2, NT, preferred_element_type=F32)
            prev = jnp.where(g == 0, 0.0, at_s[qb % 2])
            at_s[qb % 2] = prev + contrib

        def tree(tl, op):
            while len(tl) > 1:
                tl = [op(tl[i], tl[i + 1]) if i + 1 < len(tl) else tl[i] for i in range(0, len(tl), 2)]
            return tl[0]

        def qk(qh, g, s_ref):
            mx = None
            for c in range(S // QCK):
                s = lax.dot_general(qh, k_v[g, pl.ds(c * QCK, QCK), :], NT, preferred_element_type=F32)
                s_ref[:, pl.ds(c * QCK, QCK)] = s
                tl = [s[:, t * 128:(t + 1) * 128] for t in range(QCK // 128)]
                if mxmode == 'tree':
                    tl = [tree(tl, jnp.maximum)]
                for st in tl:
                    mx = st if mx is None else jnp.maximum(mx, st)
            return jnp.max(mx, axis=-1, keepdims=True)

        def pv_raw(g, s_ref, m):
            acc = None
            ls = None
            for c in range(S // CK):
                p = jnp.exp2(s_ref[:, pl.ds(c * CK, CK)] - m)
                tl = [p[:, t * 128:(t + 1) * 128] for t in range(CK // 128)]
                if lsmode == 'tree':
                    tl = [tree(tl, jnp.add)]
                elif lsmode == 'pair':
                    tl = [tl[i] + tl[i + 1] for i in range(0, len(tl), 2)]
                for pt in tl:
                    ls = pt if ls is None else ls + pt
                d = jnp.dot(p.astype(BF), v_v[g, pl.ds(c * CK, CK), :], preferred_element_type=F32)
                acc = d if acc is None else acc + d
            return acc, ls

        def epilogue1(qb):
            c0 = pl.multiple_of(qb * BQ, BQ)
            x = xT_v[:, pl.ds(c0, BQ)].astype(F32)
            x1b = (x + tab(2) * (at_s[qb % 2] if 'noat' not in DBG else tab(0))).astype(BF)
            x1 = x1b.astype(F32)
            mean, _, var = _ln_stats_t(x1)
            if 'rsq' in DBG: return x1, _rnd(mean), lax.rsqrt(var + EPS_BF16)
            den = _rnd(jnp.sqrt(_rnd(_rnd(var) + EPS_BF16)))
            return x1, _rnd(mean), 1.0 / den

        def epilogue2(qb, x1, mean, inv):
            c0 = pl.multiple_of(qb * BQ, BQ)
            y = _rnd(_rnd(x1 - mean) * inv)
            h2b = (_rnd(y * tab(4)) + tab(3)).astype(BF)
            h2 = h2b.astype(F32)
            h2_s[:, pl.ds(c0, BQ)] = h2b
            if rmxu:
                r = jnp.dot(wrb_s[...], h2b, preferred_element_type=F32)[0:1, :]
            else:
                r = jnp.sum(h2 * tab(6), axis=0, keepdims=True)
            r_s[pl.ds(qb, 1), :] = _rnd(r)
            out_s[:, pl.ds(c0, BQ)] = (x1 + tab(5) * h2).astype(BF)
            return r

        def epilogue(qb):
            epilogue2(qb, *epilogue1(qb))

        def gate(m, tok):
            t = jnp.max(tok, axis=1, keepdims=True)
            never = jnp.logical_and(t != t, t == t)
            return jnp.where(never, 0.0, m)

        _s.__exit__(None, None, None); _s = scope('pro_ln'); _s.__enter__()
        with scope('w_x0'):
            cp_x0.wait()
        if early == 1:
            cp_q(0).start()
            cp_k(0).start()
            cp_v(0).start()

        def tables_a():
            with scope('w_c'):
                cp_c.wait()
            cf = c_v[...].astype(F32)
            sc = _rnd(cf * _rnd(jax.nn.sigmoid(cf)))
            sc16 = jnp.broadcast_to(sc, (16, D)).astype(BF)
            with scope('w_wma'):
                for cp in cp_wma:
                    cp.wait()
            if early == 2:
                cp_q(0).start()
                cp_k(0).start()
                cp_v(0).start()
            cp_q(1).start()
            cp_k(1).start()
            cp_v(1).start()
            moda = _rnd(jnp.dot(sc16, wm_v[:, 0:WA], preferred_element_type=F32)[0:1, :])
            ta = col_table(moda)
            tab_s[0 * D:1 * D, :] = ta[0:D]
            tab_s[1 * D:2 * D, :] = _rnd(1.0 + ta[D:2 * D])
        ln1(0, tables_a)
        with scope('w_q0'):
            cp_q(0).wait()
        qproj(0, 0, 0)

        def unit(qb, g, qbn, gn, qbp, gp, special, skip=''):
            slots = orders[{None: 0, 'A': 1, 'C': 2}[special]].split(',')
            toks = {}
            slot = g % 2

            def fill(i):
                for ch in slots[i]:
                    if ch in skip:
                        continue
                    if ch == 'q':
                        qproj(qbn, gn, 1 - slot)
                    elif ch == 'a':
                        qproj_half(qbn, gn, 1 - slot, 0)
                    elif ch == 'b':
                        qproj_half(qbn, gn, 1 - slot, 1)
                    elif ch == 'r':
                        qproj_rows(qbn, gn, 1 - slot, 0)
                    elif ch == 's':
                        qproj_rows(qbn, gn, 1 - slot, 1)
                    elif ch == 'x':
                        oproj_half(qbp, gp, 0)
                    elif ch == 'y':
                        oproj_half(qbp, gp, 1)
                    elif ch == 'o':
                        oproj(qbp, gp)
                    elif ch == 'e':
                        toks['e'] = epilogue1(qb - 1)
                    elif ch == 'f':
                        toks['f'] = epilogue2(qb - 1, *toks['e'])
                    elif ch == 'n':
                        ln1(qbn)
            HB = BQ // RS
            sref = [s_a.at[0], s_b.at[0]]
            if RS == 1:
                res = []
                for j in range(2):
                    fill(3 * j)
                    m = qk(q_s[slot, :, j * 128:(j + 1) * 128], g, sref[j])
                    fill(3 * j + 1)
                    res.append(pv_raw(g, sref[j], m))
                    fill(3 * j + 2)
                for j in range(2):
                    acc_s[j] = res[j][0]
                    ls_s[j] = res[j][1]
            else:
                ms = {}
                res = {}
                for st in sched.split():
                    if st[0] == 'f':
                        fill(int(st[1]))
                        continue
                    j = int(st[1]); r = int(st[2])
                    rows = slice(r * HB, (r + 1) * HB)
                    if st[0] == 'Q':
                        ms[j, r] = qk(q_s[slot, rows, j * 128:(j + 1) * 128], g, sref[j].at[rows])
                    else:
                        a, l = pv_raw(g, sref[j].at[rows], ms[j, r])
                        acc_s[j, rows] = a
                        ls_s[j, rows] = l

        def first_body(g, carry, peeled=False):
            with scope('w_kvq'):
                cp_k(g).wait()
                cp_v(g).wait()
                cp_q(g + 1).wait()

            if peeled:
                cp_q(2).start()
                cp_k(2).start()
                cp_v(2).start()
                cp_o(0).start()
                with scope('bodyFirst'):
                    unit(0, 0, 0, 1, 0, 0, None, skip='o')
                return carry
            cp_o(g - 1).wait()

            @pl.when(g + 2 < HKV)
            def _():
                cp_q(g + 2).start()
                cp_k(g + 2).start()
                cp_v(g + 2).start()
            cp_o(g).start()

            @pl.when(g == 3)
            def _():
                cp_xr.start()
                cp_wmb.start()
                cp_wr.start()

            @pl.when(g == 10)
            def _():
                cp_xr.wait()
                cp_wmb.wait()
                cp_wr.wait()
                with scope('tables_b'):
                    tables_b()

            @pl.when(g == HKV - 2)
            def _():
                cp_o(HKV - 1).start()
            with scope('bodyG0'):
                unit(0, g, 0, g + 1, 0, g - 1, None)
            return carry

        _s.__exit__(None, None, None); _s = scope('loop0'); _s.__enter__()
        first_body(0, 0, peeled=True)
        lax.fori_loop(1, HKV - 1, first_body, 0)
        cp_k(HKV - 1).wait()
        cp_v(HKV - 1).wait()
        cp_o(HKV - 2).wait()
        cp_o(HKV - 1).wait()
        cp_wg.start()
        cp_wu.start()
        cp_wd.start()
        _s.__exit__(None, None, None); _s = scope('loop'); _s.__enter__()

        def gen(nb, g):
            with scope('bodyG'):
                unit(nb, g, nb, g + 1, nb, g - 1, None)

        def block_body(qb, carry):
            nb = qb + 1
            with scope('bodyC'):
                unit(qb, HKV - 1, nb, 0, qb, HKV - 2, 'C')

            def inner(g, c2):
                first = g == 0
                with scope('bodyG'):
                    unit(nb, g, nb, g + 1, jnp.where(first, qb, nb), jnp.where(first, HKV - 1, g - 1), None)

                @pl.when(first)
                def _():
                    with scope('epi'):
                        epilogue(qb)
                    cp_out(qb).start()
                return c2
            lax.fori_loop(0, HKV - 1, inner, 0)
            return carry

        lax.fori_loop(0, NQB - 1, block_body, 0)
        with scope('bodyL'):
            unit(NQB - 1, HKV - 1, 0, 0, NQB - 1, HKV - 2, None, skip='q')
        _s.__exit__(None, None, None); _s = scope('t_epi'); _s.__enter__()
        oproj(NQB - 1, HKV - 1)
        epilogue(NQB - 1)
        cp_out(NQB - 1).start()

        _s.__exit__(None, None, None); _s = scope('t_top'); _s.__enter__()
        r = r_s[...] + 0.0
        pos = lax.broadcasted_iota(I32, (NQB, BQ), 0) * BQ + lax.broadcasted_iota(I32, (NQB, BQ), 1)
        b16 = lax.shift_right_logical(pltpu.bitcast(r, I32), 16)
        o16 = jnp.where(b16 >= 0x8000, 0xFFFF - b16, b16 + 0x8000)
        o16 = jnp.where(r != r, 0, o16)
        key = pltpu.bitcast(0x10000000 | (o16 << 11) | (S - 1 - pos), F32)
        rowc = lax.broadcasted_iota(I32, (16, 1), 0)
        rsel = jnp.zeros((16, 1), F32)
        idxs = []
        for i in range(C):
            m = jnp.max(jnp.max(key, axis=1, keepdims=True), axis=0, keepdims=True)
            key = jnp.where(key == m, 0.0, key)
            mb = pltpu.bitcast(m, I32)
            idx = (S - 1) - (mb & (S - 1))
            o = lax.shift_right_logical(mb, 11) & 0xFFFF
            rb = jnp.where(o >= 0x8000, o - 0x8000, 0xFFFF - o)
            rv = pltpu.bitcast(rb << 16, F32)
            rsel = jnp.where(rowc == i, rv, rsel)
            idxs.append(idx[0, 0])
        tiles = []
        lanes = []
        xs = None
        row16 = lax.broadcasted_iota(I32, (16, 128), 0)
        lane16 = lax.broadcasted_iota(I32, (16, 128), 1)
        for i in range(C):
            ii = jnp.clip(idxs[i], 0, S - 1)
            t = ii // 128
            ln = ii % 128
            tiles.append(t)
            lanes.append(ln)
            oh = jnp.where(jnp.logical_and(row16 == i, lane16 == ln), 1.0, 0.0).astype(BF)
            c0 = pl.multiple_of(t * 128, 128)
            part = lax.dot_general(oh, h2_s[:, pl.ds(c0, 128)], NT, preferred_element_type=F32)
            xs = part if xs is None else xs + part
        xsb = xs.astype(BF)
        _s.__exit__(None, None, None); _s = scope('t_ffn'); _s.__enter__()
        cp_wg.wait()
        cp_wu.wait()
        cp_wd.wait()
        gt = _rnd(jnp.dot(xsb, wg_v[...], preferred_element_type=F32))
        gg = _rnd(gt * _rnd(jax.nn.sigmoid(gt)))
        uu = _rnd(jnp.dot(xsb, wu_v[...], preferred_element_type=F32))
        a = (gg * uu).astype(BF)
        y = _rnd(lax.dot_general(a, wdT_v[...], NT, preferred_element_type=F32))
        _s.__exit__(None, None, None); _s = scope('t_new'); _s.__enter__()
        y = _rnd(y * _rnd(jax.nn.sigmoid(rsel)))
        delta = y * jnp.broadcast_to(gb_s[0:1, :], (16, D))
        deltaT = jnp.concatenate([delta, jnp.zeros((128 - 16, D), F32)], axis=0).T
        _s.__exit__(None, None, None); _s = scope('t_patch'); _s.__enter__()
        for qb in range(NQB):
            cp_out(qb).wait()
        lane128 = lax.broadcasted_iota(I32, (D, 128), 1)
        moved = [pltpu.roll(deltaT, (lanes[i] - i) % 128, axis=1) for i in range(C)]

        def tile_cp(i):
            c0 = pl.multiple_of(tiles[i] * 128, 128)
            return pltpu.make_async_copy(out_s.at[:, pl.ds(c0, 128)], o_hbm.at[:, pl.ds(c0, 128)], ksem.at[i])

        def last_in_tile(i):
            ok = tiles[i] == tiles[i]
            for j in range(i + 1, C):
                ok = jnp.logical_and(ok, tiles[j] != tiles[i])
            return ok
        for i in range(C):
            c0 = pl.multiple_of(tiles[i] * 128, 128)
            cur = out_s[:, pl.ds(c0, 128)].astype(F32)
            out_s[:, pl.ds(c0, 128)] = (cur + jnp.where(lane128 == lanes[i], moved[i], 0.0)).astype(BF)
            pl.when(last_in_tile(i))(lambda i=i: tile_cp(i).start())
        for i in range(C):
            pl.when(last_in_tile(i))(lambda i=i: tile_cp(i).wait())
        _s.__exit__(None, None, None)

    return kernel


def run(A_x, A_k_cache, A_v_cache, A_wq, A_wo, B_x, B_w_r, B_w_gate, B_w_up, B_w_down, c, w_mod,
        BQ=512, CK=512, flags=None, orders=('q,,,,,o', 'efq,,,,,o', ',nq,,,,o'), reps=0, fuse=False, gate_j=0, opaque=False, pair=False, split=True, QCK=512, mxmode='seq', lsmode='tree', rmxu=False, NSPL=1, early=1, RS=1, sched=''):
    xT = A_x.reshape(S, D).T
    k = A_k_cache.reshape(HKV, S, DH)
    v = A_v_cache.reshape(HKV, S, DH)
    wr = B_w_r.reshape(1, D)
    NQB = S // BQ
    any_spec = pl.BlockSpec(memory_space=pl.ANY)
    outT = pl.pallas_call(
        make_kernel(BQ, CK, orders, reps, fuse, gate_j, opaque, pair, split, QCK, mxmode, lsmode, rmxu, NSPL, early, RS, sched),
        in_specs=[any_spec] * 11,
        out_specs=any_spec,
        out_shape=jax.ShapeDtypeStruct((D, S), BF),
        scratch_shapes=[
            pltpu.VMEM((D, S), BF),
            pltpu.VMEM((HKV, S, DH), BF),
            pltpu.VMEM((HKV, S, DH), BF),
            pltpu.VMEM((D, HQ * DH), BF),
            pltpu.VMEM((D, HQ * DH), BF),
            pltpu.VMEM((1, D), BF),
            pltpu.VMEM((D, F), BF),
            pltpu.VMEM((D, F), BF),
            pltpu.VMEM((D, F), BF),
            pltpu.VMEM((1, D), BF),
            pltpu.VMEM((D, 6 * D), BF),
            pltpu.VMEM((7 * D, 128), F32),
            pltpu.VMEM((8, D), F32),
            pltpu.VMEM((16, D), BF),
            pltpu.VMEM((2, BQ, D), BF),
            pltpu.VMEM((2, BQ, 256), BF),
            pltpu.VMEM((2, BQ, S), F32),
            pltpu.VMEM((2, BQ, S), F32),
            pltpu.SMEM((1,), I32),
            pltpu.VMEM((2, BQ, 128), F32),
            pltpu.VMEM((2, BQ, 128), F32),
            pltpu.VMEM((2, D, BQ), F32),
            pltpu.VMEM((D, S), BF),
            pltpu.VMEM((D, S), BF),
            pltpu.VMEM((NQB, BQ), F32),
            pltpu.SemaphoreType.DMA((9,)),
            pltpu.SemaphoreType.DMA((HKV,)),
            pltpu.SemaphoreType.DMA((HKV,)),
            pltpu.SemaphoreType.DMA((HKV,)),
            pltpu.SemaphoreType.DMA((HKV,)),
            pltpu.SemaphoreType.DMA((NQB,)),
            pltpu.SemaphoreType.DMA((NSPL,)),
        ],
        compiler_params=pltpu.CompilerParams(vmem_limit_bytes=110 * 1024 * 1024, flags=flags),
    )(xT, k, v, A_wq, A_wo.T, wr, B_w_gate, B_w_up, B_w_down.T, c, w_mod)
    return outT.T.reshape(1, S, D)


@jax.jit
def pallas_adaLN_cond__gqa_block_cached__moe_arch_mod__prompt_kernel(
    A_x: jax.Array,
    A_k_cache: jax.Array,
    A_v_cache: jax.Array,
    A_wq: jax.Array,
    A_wo: jax.Array,
    B_x: jax.Array,
    B_w_r: jax.Array,
    B_w_gate: jax.Array,
    B_w_up: jax.Array,
    B_w_down: jax.Array,
    c: jax.Array,
    w_mod: jax.Array,
):
    return run(A_x, A_k_cache, A_v_cache, A_wq, A_wo, B_x, B_w_r, B_w_gate, B_w_up, B_w_down, c, w_mod)
```

```python
import jax
import jax.numpy as jnp
from jax import lax
import jax.experimental.pallas as pl
import jax.experimental.pallas.tpu as pltpu

S = 2048
D = 576
HKV = 16
DH = 128
F = 4608
C = 8
BQ = 512
CK = 512
THR = 17
NQB = S // BQ
NL = BQ // 128
WA = 2 * D

EPS = 1e-5
EPS_BF16 = 1.0013580322265625e-05
QSCALE = DH ** -0.5 * 1.4426950408889634

BF = jnp.bfloat16
F32 = jnp.float32
I32 = jnp.int32
NT = (((1,), (1,)), ((), ()))


def _rnd(x):
    return x.astype(BF).astype(F32)


def _ln_stats(x):
    mean = jnp.sum(x, axis=0, keepdims=True) * (1.0 / D)
    xc = x - mean
    var = jnp.sum(xc * xc, axis=0, keepdims=True) * (1.0 / D)
    return mean, xc, var


def _col_table(row):
    return jnp.broadcast_to(row, (128, row.shape[1])).T


def _tree_sum(parts):
    while len(parts) > 1:
        parts = [parts[i] + parts[i + 1] for i in range(0, len(parts), 2)]
    return parts[0]


def _kernel(xT_hbm, k_hbm, v_hbm, wq_hbm, woT_hbm, wr_hbm, wg_hbm, wu_hbm, wdT_hbm, c_hbm, wm_hbm,
            o_hbm,
            xT_v, k_v, v_v, wq_v, woT_v, wr_v, wg_v, wu_v, wdT_v, c_v, wm_v,
            tab_s, gb_s, h_s, q_s, s_s, acc_s, ls_s, at_s, h2_s, out_s, r_s,
            sems, ksem, vsem, qsem, osem, outsem):
    cp_c = pltpu.make_async_copy(c_hbm, c_v, sems.at[0])
    cp_wma = pltpu.make_async_copy(wm_hbm.at[:, pl.ds(0, WA)], wm_v.at[:, pl.ds(0, WA)], sems.at[1])
    cp_wmb = pltpu.make_async_copy(wm_hbm.at[:, pl.ds(WA, 6 * D - WA)], wm_v.at[:, pl.ds(WA, 6 * D - WA)],
                                   sems.at[2])
    cp_x0 = pltpu.make_async_copy(xT_hbm.at[:, pl.ds(0, BQ)], xT_v.at[:, pl.ds(0, BQ)], sems.at[3])
    cp_xr = pltpu.make_async_copy(xT_hbm.at[:, pl.ds(BQ, S - BQ)], xT_v.at[:, pl.ds(BQ, S - BQ)], sems.at[4])
    cp_wr = pltpu.make_async_copy(wr_hbm, wr_v, sems.at[5])
    cp_wg = pltpu.make_async_copy(wg_hbm, wg_v, sems.at[6])
    cp_wu = pltpu.make_async_copy(wu_hbm, wu_v, sems.at[7])
    cp_wd = pltpu.make_async_copy(wdT_hbm, wdT_v, sems.at[8])

    def cp_k(g):
        return pltpu.make_async_copy(k_hbm.at[g], k_v.at[g], ksem.at[g])

    def cp_v(g):
        return pltpu.make_async_copy(v_hbm.at[g], v_v.at[g], vsem.at[g])

    def cp_q(g):
        c0 = pl.multiple_of(g * 256, 256)
        return pltpu.make_async_copy(wq_hbm.at[:, pl.ds(c0, 256)], wq_v.at[:, pl.ds(c0, 256)], qsem.at[g])

    def cp_o(g):
        c0 = pl.multiple_of(g * 256, 256)
        return pltpu.make_async_copy(woT_hbm.at[:, pl.ds(c0, 256)], woT_v.at[:, pl.ds(c0, 256)], osem.at[g])

    def cp_out(qb):
        c0 = pl.multiple_of(qb * BQ, BQ)
        return pltpu.make_async_copy(out_s.at[:, pl.ds(c0, BQ)], o_hbm.at[:, pl.ds(c0, BQ)], outsem.at[qb])

    def silu_c():
        cf = c_v[...].astype(F32)
        sc = _rnd(cf * _rnd(jax.nn.sigmoid(cf)))
        return jnp.broadcast_to(sc, (16, D)).astype(BF)

    def tables_a():
        cp_c.wait()
        sc16 = silu_c()
        cp_wma.wait()
        moda = _rnd(jnp.dot(sc16, wm_v[:, 0:WA], preferred_element_type=F32)[0:1, :])
        ta = _col_table(moda)
        tab_s[0 * D:1 * D, :] = ta[0:D]
        tab_s[1 * D:2 * D, :] = _rnd(1.0 + ta[D:2 * D])

    def tables_b():
        modb = _rnd(jnp.dot(silu_c(), wm_v[:, WA:6 * D], preferred_element_type=F32)[0:8, :])
        gb_s[...] = modb[:, 3 * D:4 * D]
        tb = _col_table(modb[0:1, :])
        tab_s[2 * D:3 * D, :] = tb[0:D]
        tab_s[3 * D:4 * D, :] = tb[D:2 * D]
        tab_s[4 * D:5 * D, :] = _rnd(1.0 + tb[2 * D:3 * D])
        tab_s[5 * D:6 * D, :] = tb[3 * D:4 * D]
        tab_s[6 * D:7 * D, :] = _col_table(wr_v[...].reshape(1, D).astype(F32))

    def tab(i):
        return jnp.concatenate([tab_s[i * D:(i + 1) * D, :]] * NL, axis=1)

    def ln1(qb, mid=None):
        c0 = pl.multiple_of(qb * BQ, BQ)
        x = xT_v[:, pl.ds(c0, BQ)].astype(F32)
        _, xc, var = _ln_stats(x)
        inv = lax.rsqrt(var + EPS)
        if mid is not None:
            mid()
        h_s[qb % 2] = (xc * inv * tab(1) + tab(0)).astype(BF).T

    def qproj(qb, g, slot, rows=slice(None)):
        c0 = pl.multiple_of(g * 256, 256)
        q = jnp.dot(h_s[qb % 2, rows], wq_v[:, pl.ds(c0, 256)], preferred_element_type=F32)
        q_s[slot, rows] = (q * QSCALE).astype(BF)

    def norm(j):
        l = jnp.sum(ls_s[j], axis=-1, keepdims=True)
        r0 = pltpu.reciprocal(l, approx=True)
        return (acc_s[j] * (r0 * (2.0 - l * r0))).astype(BF)

    def oproj(qb, g):
        c0 = pl.multiple_of(g * 256, 256)
        o2 = jnp.concatenate([norm(0), norm(1)], axis=1)
        contrib = lax.dot_general(woT_v[:, pl.ds(c0, 256)], o2, NT, preferred_element_type=F32)
        prev = jnp.where(g == 0, 0.0, at_s[qb % 2])
        at_s[qb % 2] = prev + contrib

    def scores(qh, g, s_ref):
        mx = None
        for c in range(S // CK):
            s = lax.dot_general(qh, k_v[g, pl.ds(c * CK, CK), :], NT, preferred_element_type=F32)
            s_ref[:, pl.ds(c * CK, CK)] = s
            for t in range(CK // 128):
                st = s[:, t * 128:(t + 1) * 128]
                mx = st if mx is None else jnp.maximum(mx, st)
        return jnp.max(mx, axis=-1, keepdims=True)

    def softmax_pv(g, s_ref, m):
        mb = jnp.broadcast_to(m, (BQ, 128))
        acc = ls = prev = None
        for c in range(S // CK):
            mg = mb
            if prev is not None:
                tok = jnp.concatenate([prev[THR * 16:]] + [prev[BQ - 16:]] * THR, axis=0)
                never = jnp.logical_and(tok != tok, tok == tok)
                mg = jnp.where(never, 0.0, mb)
            tl = [jnp.exp2(s_ref[:, pl.ds(c * CK + t * 128, 128)] - mg) for t in range(CK // 128)]
            p = jnp.concatenate(tl, axis=1)
            pt = _tree_sum(tl)
            ls = pt if ls is None else ls + pt
            prev = jnp.dot(p.astype(BF), v_v[g, pl.ds(c * CK, CK), :], preferred_element_type=F32)
            acc = prev if acc is None else acc + prev
        return acc, ls

    def epilogue(qb):
        c0 = pl.multiple_of(qb * BQ, BQ)
        x = xT_v[:, pl.ds(c0, BQ)].astype(F32)
        x1 = _rnd(x + tab(2) * at_s[qb % 2])
        mean, _, var = _ln_stats(x1)
        den = _rnd(jnp.sqrt(_rnd(_rnd(var) + EPS_BF16)))
        y = _rnd(_rnd(x1 - _rnd(mean)) * (1.0 / den))
        h2b = (_rnd(y * tab(4)) + tab(3)).astype(BF)
        h2 = h2b.astype(F32)
        h2_s[:, pl.ds(c0, BQ)] = h2b
        r_s[pl.ds(qb, 1), :] = _rnd(jnp.sum(h2 * tab(6), axis=0, keepdims=True))
        out_s[:, pl.ds(c0, BQ)] = (x1 + tab(5) * h2).astype(BF)

    def unit(g, nxt=None, prv=None, new_block=False):
        slot = g % 2
        half = BQ // 2
        if new_block:
            ln1(nxt[0])
        elif nxt is not None:
            qproj(nxt[0], nxt[1], 1 - slot)
        res = []
        for j in range(2):
            m = scores(q_s[slot, :, j * 128:(j + 1) * 128], g, s_s.at[j])
            if new_block:
                qproj(nxt[0], nxt[1], 1 - slot, slice(j * half, (j + 1) * half))
            res.append(softmax_pv(g, s_s.at[j], m))
        if prv is not None:
            oproj(*prv)
        for j in range(2):
            acc_s[j] = res[j][0]
            ls_s[j] = res[j][1]

    cp_x0.start()
    cp_c.start()
    cp_wma.start()
    cp_x0.wait()
    cp_q(0).start()
    cp_k(0).start()
    cp_v(0).start()

    def mid():
        tables_a()
        cp_q(1).start()
        cp_k(1).start()
        cp_v(1).start()
    ln1(0, mid)
    cp_q(0).wait()
    qproj(0, 0, 0)

    cp_k(0).wait()
    cp_v(0).wait()
    cp_q(1).wait()
    cp_q(2).start()
    cp_k(2).start()
    cp_v(2).start()
    cp_o(0).start()
    unit(0, nxt=(0, 1))

    def first_block(g, carry):
        cp_k(g).wait()
        cp_v(g).wait()
        cp_q(g + 1).wait()
        cp_o(g - 1).wait()

        @pl.when(g + 2 < HKV)
        def _():
            cp_q(g + 2).start()
            cp_k(g + 2).start()
            cp_v(g + 2).start()
        cp_o(g).start()

        @pl.when(g == 3)
        def _():
            cp_xr.start()
            cp_wmb.start()
            cp_wr.start()

        @pl.when(g == 10)
        def _():
            cp_xr.wait()
            cp_wmb.wait()
            cp_wr.wait()
            tables_b()

        @pl.when(g == HKV - 2)
        def _():
            cp_o(HKV - 1).start()
        unit(g, nxt=(0, g + 1), prv=(0, g - 1))
        return carry

    lax.fori_loop(1, HKV - 1, first_block, 0)
    cp_k(HKV - 1).wait()
    cp_v(HKV - 1).wait()
    cp_o(HKV - 2).wait()
    cp_o(HKV - 1).wait()
    cp_wg.start()
    cp_wu.start()
    cp_wd.start()

    def block(qb, carry):
        nb = qb + 1
        unit(HKV - 1, nxt=(nb, 0), prv=(qb, HKV - 2), new_block=True)

        def inner(g, c2):
            first = g == 0
            unit(g, nxt=(nb, g + 1), prv=(jnp.where(first, qb, nb), jnp.where(first, HKV - 1, g - 1)))
            return c2
        lax.fori_loop(0, HKV - 1, inner, 0)
        epilogue(qb)
        cp_out(qb).start()
        return carry

    lax.fori_loop(0, NQB - 1, block, 0)
    unit(HKV - 1, prv=(NQB - 1, HKV - 2))
    oproj(NQB - 1, HKV - 1)
    epilogue(NQB - 1)
    cp_out(NQB - 1).start()

    r = r_s[...] + 0.0
    pos = lax.broadcasted_iota(I32, (NQB, BQ), 0) * BQ + lax.broadcasted_iota(I32, (NQB, BQ), 1)
    b16 = lax.shift_right_logical(pltpu.bitcast(r, I32), 16)
    o16 = jnp.where(b16 >= 0x8000, 0xFFFF - b16, b16 + 0x8000)
    o16 = jnp.where(r != r, 0, o16)
    key = pltpu.bitcast(0x10000000 | (o16 << 11) | (S - 1 - pos), F32)
    rowc = lax.broadcasted_iota(I32, (16, 1), 0)
    rsel = jnp.zeros((16, 1), F32)
    idxs = []
    for i in range(C):
        m = jnp.max(jnp.max(key, axis=1, keepdims=True), axis=0, keepdims=True)
        key = jnp.where(key == m, 0.0, key)
        mb = pltpu.bitcast(m, I32)
        o = lax.shift_right_logical(mb, 11) & 0xFFFF
        rb = jnp.where(o >= 0x8000, o - 0x8000, 0xFFFF - o)
        rsel = jnp.where(rowc == i, pltpu.bitcast(rb << 16, F32), rsel)
        idxs.append(((S - 1) - (mb & (S - 1)))[0, 0])

    tiles, lanes = [], []
    xs = None
    row16 = lax.broadcasted_iota(I32, (16, 128), 0)
    lane16 = lax.broadcasted_iota(I32, (16, 128), 1)
    for i in range(C):
        ii = jnp.clip(idxs[i], 0, S - 1)
        tiles.append(ii // 128)
        lanes.append(ii % 128)
        oh = jnp.where(jnp.logical_and(row16 == i, lane16 == lanes[i]), 1.0, 0.0).astype(BF)
        c0 = pl.multiple_of(tiles[i] * 128, 128)
        part = lax.dot_general(oh, h2_s[:, pl.ds(c0, 128)], NT, preferred_element_type=F32)
        xs = part if xs is None else xs + part
    xsb = xs.astype(BF)

    cp_wg.wait()
    cp_wu.wait()
    cp_wd.wait()
    gt = _rnd(jnp.dot(xsb, wg_v[...], preferred_element_type=F32))
    gg = _rnd(gt * _rnd(jax.nn.sigmoid(gt)))
    uu = _rnd(jnp.dot(xsb, wu_v[...], preferred_element_type=F32))
    a = (gg * uu).astype(BF)
    y = _rnd(lax.dot_general(a, wdT_v[...], NT, preferred_element_type=F32))
    y = _rnd(y * _rnd(jax.nn.sigmoid(rsel)))
    delta = y * jnp.broadcast_to(gb_s[0:1, :], (16, D))
    deltaT = jnp.concatenate([delta, jnp.zeros((128 - 16, D), F32)], axis=0).T

    for qb in range(NQB):
        cp_out(qb).wait()
    lane128 = lax.broadcasted_iota(I32, (D, 128), 1)
    moved = [jnp.where(lane128 == lanes[i], pltpu.roll(deltaT, (lanes[i] - i) % 128, axis=1), 0.0)
             for i in range(C)]

    def tile_cp(i):
        c0 = pl.multiple_of(tiles[i] * 128, 128)
        return pltpu.make_async_copy(out_s.at[:, pl.ds(c0, 128)], o_hbm.at[:, pl.ds(c0, 128)], ksem.at[i])

    def last_in_tile(i):
        ok = tiles[i] == tiles[i]
        for j in range(i + 1, C):
            ok = jnp.logical_and(ok, tiles[j] != tiles[i])
        return ok

    for i in range(C):
        c0 = pl.multiple_of(tiles[i] * 128, 128)
        cur = out_s[:, pl.ds(c0, 128)].astype(F32)
        out_s[:, pl.ds(c0, 128)] = (cur + moved[i]).astype(BF)
        pl.when(last_in_tile(i))(lambda i=i: tile_cp(i).start())
    for i in range(C):
        pl.when(last_in_tile(i))(lambda i=i: tile_cp(i).wait())


def run(A_x, A_k_cache, A_v_cache, A_wq, A_wo, B_x, B_w_r, B_w_gate, B_w_up, B_w_down, c, w_mod):
    del B_x
    outT = pl.pallas_call(
        _kernel,
        in_specs=[pl.BlockSpec(memory_space=pl.ANY)] * 11,
        out_specs=pl.BlockSpec(memory_space=pl.ANY),
        out_shape=jax.ShapeDtypeStruct((D, S), BF),
        scratch_shapes=[
            pltpu.VMEM((D, S), BF),
            pltpu.VMEM((HKV, S, DH), BF),
            pltpu.VMEM((HKV, S, DH), BF),
            pltpu.VMEM((D, 2 * HKV * DH), BF),
            pltpu.VMEM((D, 2 * HKV * DH), BF),
            pltpu.VMEM((D,), BF),
            pltpu.VMEM((D, F), BF),
            pltpu.VMEM((D, F), BF),
            pltpu.VMEM((D, F), BF),
            pltpu.VMEM((1, D), BF),
            pltpu.VMEM((D, 6 * D), BF),
            pltpu.VMEM((7 * D, 128), F32),
            pltpu.VMEM((8, D), F32),
            pltpu.VMEM((2, BQ, D), BF),
            pltpu.VMEM((2, BQ, 256), BF),
            pltpu.VMEM((2, BQ, S), F32),
            pltpu.VMEM((2, BQ, 128), F32),
            pltpu.VMEM((2, BQ, 128), F32),
            pltpu.VMEM((2, D, BQ), F32),
            pltpu.VMEM((D, S), BF),
            pltpu.VMEM((D, S), BF),
            pltpu.VMEM((NQB, BQ), F32),
            pltpu.SemaphoreType.DMA((9,)),
            pltpu.SemaphoreType.DMA((HKV,)),
            pltpu.SemaphoreType.DMA((HKV,)),
            pltpu.SemaphoreType.DMA((HKV,)),
            pltpu.SemaphoreType.DMA((HKV,)),
            pltpu.SemaphoreType.DMA((NQB,)),
        ],
        compiler_params=pltpu.CompilerParams(vmem_limit_bytes=110 * 1024 * 1024),
    )(A_x.reshape(S, D).T, A_k_cache.reshape(HKV, S, DH), A_v_cache.reshape(HKV, S, DH), A_wq, A_wo.T,
      B_w_r, B_w_gate, B_w_up, B_w_down.T, c, w_mod)
    return outT.T.reshape(1, S, D)


@jax.jit
def pallas_adaLN_cond__gqa_block_cached__moe_arch_mod__prompt_kernel(
    A_x: jax.Array,
    A_k_cache: jax.Array,
    A_v_cache: jax.Array,
    A_wq: jax.Array,
    A_wo: jax.Array,
    B_x: jax.Array,
    B_w_r: jax.Array,
    B_w_gate: jax.Array,
    B_w_up: jax.Array,
    B_w_down: jax.Array,
    c: jax.Array,
    w_mod: jax.Array,
):
    return run(A_x, A_k_cache, A_v_cache, A_wq, A_wo, B_x, B_w_r, B_w_gate, B_w_up, B_w_down, c, w_mod)
```
